```python
import jax
import jax.numpy as jnp

def _softmax(x, axis=-1):
    return jax.nn.softmax(x, axis=axis)
def _gelu(x):
    return jax.nn.gelu(x, approximate=True)
def _silu(x):
    return jax.nn.silu(x)
def _sigmoid(x):
    return jax.nn.sigmoid(x)
def _layernorm(x, axis=-1, eps=1e-5):
    m = jnp.mean(x, axis=axis, keepdims=True)
    v = jnp.var(x, axis=axis, keepdims=True)
    return (x - m) / jnp.sqrt(v + eps)
def _scatter_add(tgt, idx, src, axis=0):
    return tgt.at[idx].add(src)
def _segment_sum(src, seg, n):
    return jax.ops.segment_sum(src, seg, n)
class _Rng:
    def __init__(self, key):
        self._k = key
    def _next(self):
        self._k, sub = jax.random.split(self._k)
        return sub
    def normal(self, shape):
        return jax.random.normal(self._next(), shape, dtype=jnp.bfloat16)
    def randint(self, lo, hi, shape):
        return jax.random.randint(self._next(), shape, lo, hi, dtype=jnp.int32)
    def uniform(self, shape, lo=0.0, hi=1.0):
        return jax.random.uniform(self._next(), shape, jnp.bfloat16, lo, hi)
    def permutation(self, n):
        return jax.random.permutation(self._next(), n)


kernel_name = 'gated_mix__ssm_conv_h3__sliding_local_dilated__prompt'

def setup_inputs():
    _rng = _Rng(jax.random.key(int.from_bytes(__import__("os").urandom(4), "little")))
    _w = (lambda a: (lambda t: t.astype(jnp.bfloat16) if jnp.issubdtype(t.dtype, jnp.floating) else t)(jnp.asarray(a)))
    def _A_setup():
        B, S, D = 1, 2048, 640
        ks = 4
        return {
            "q": _w((lambda *s: _rng.normal(s) * 0.05)(B, S, D)),
            "k": _w((lambda *s: _rng.normal(s) * 0.05)(B, S, D)),
            "v": _w((lambda *s: _rng.normal(s) * 0.05)(B, S, D)),
            "shift_k": _w((lambda *s: _rng.normal(s) * 0.05)(D, ks) * 0.5),
            "ssm_k": _w((lambda *s: _rng.normal(s) * 0.05)(D, S) * (1.0 / S ** 0.5)),
            "ssm_D": _w((lambda *s: _rng.normal(s) * 0.05)(D)),
        }
    _A_in = _A_setup()

    def _B_setup():
        B, S, D = 1, 2048, 640
        return {
            "x": _w((lambda *s: _rng.normal(s) * 0.05)(B, S, D)),
            "wqkv": _w((lambda *s: _rng.normal(s) * 0.05)(D, 3 * D)),
            "wo": _w((lambda *s: _rng.normal(s) * 0.05)(D, D)),
        }
    _B_in = _B_setup()

    return {
        "A_q": _A_in["q"],
        "A_k": _A_in["k"],
        "A_v": _A_in["v"],
        "A_shift_k": _A_in["shift_k"],
        "A_ssm_k": _A_in["ssm_k"],
        "A_ssm_D": _A_in["ssm_D"],
        "B_x": _B_in["x"],
        "B_wqkv": _B_in["wqkv"],
        "B_wo": _B_in["wo"],
        "gate_w": _w((lambda *s: _rng.normal(s) * 0.05)(640)),
    }

def reference(A_q, A_k, A_v, A_shift_k, A_ssm_k, A_ssm_D, B_x, B_wqkv, B_wo, gate_w):
    def _A_ref(q, k, v, shift_k, ssm_k, ssm_D):
        B, S, D = q.shape
        ks = shift_k.shape[-1]
        k_pad = jnp.pad(k, ((0, 0), (ks - 1, 0), (0, 0)))
        k_shift = jnp.zeros_like(k)
        for t in range(ks):
            k_shift = k_shift + k_pad[:, t:t + S, :] * shift_k[:, ks - 1 - t][None, None, :]
        kv = k_shift * v
        L = 2 * S
        kv_pad = jnp.pad(kv, ((0, 0), (0, S), (0, 0)))
        kf_pad = jnp.pad(ssm_k, ((0, 0), (0, S)))
        kv_f = (lambda x, axes=(-2,-1): jnp.fft.rfft2(x.astype(jnp.float32), axes=axes))(kv_pad[:, None, :, :], axes=(1, 2))
        kf_f = (lambda x, axes=(-2,-1): jnp.fft.rfft2(x.astype(jnp.float32), axes=axes))(kf_pad[:, None, :], axes=(1, 2))
        kf_f = (lambda x, *d: x.transpose(*d))(kf_f, 1, 2, 0)
        y_f = kv_f * kf_f[None, :, :, :]
        y = (lambda x, s, axes=(-2,-1): jnp.fft.irfft2(x, s=s, axes=axes).astype(jnp.bfloat16))(y_f, (1, L), axes=(1, 2))[:, 0, :S, :]
        y = y + kv * ssm_D[None, None, :]
        return q * y

    def _B_ref(x, wqkv, wo):
        B, S, D = x.shape
        H = 32; Dh = D // H
        W, dil = 8, 2
        qkv = (lambda x, *d: x.transpose(*d))((x @ wqkv).reshape(B, S, 3, H, Dh), 2, 0, 3, 1, 4)
        q, k, v = qkv[0], qkv[1], qkv[2]
        scale = Dh ** -0.5
        pos = jnp.arange(S)
        off = jnp.arange(W) * dil
        idx = pos[:, None] - off[None, :]
        mask = idx >= 0
        idx_c = jnp.where(mask, idx, 0).reshape(-1)
        kg = k[:, :, idx_c, :].reshape(B, H, S, W, Dh)
        vg = v[:, :, idx_c, :].reshape(B, H, S, W, Dh)
        logits = jnp.einsum("bhsd,bhswd->bhsw", q, kg) * scale
        logits = jnp.where(mask[None, None, :, :], logits, -1e9)
        attn = _softmax(logits, axis=-1)
        o = jnp.einsum("bhsw,bhswd->bhsd", attn, vg)
        return (lambda x, *d: x.transpose(*d))(o, 0, 2, 1, 3).reshape(B, S, D) @ wo

    x = A_q
    g = _sigmoid((x * gate_w).sum(-1, keepdims=True))
    a = _A_ref(x, A_k, A_v, A_shift_k, A_ssm_k, A_ssm_D)
    b = _B_ref(x, B_wqkv, B_wo)
    return g * a + (1 - g) * b
```

```python
import numpy as np
import jax
import jax.numpy as jnp
from jax import lax
from jax.experimental import pallas as pl
from jax.experimental.pallas import tpu as pltpu

S = 2048
D = 640
NT = D // 128
KS = 4
H = 32
DH = D // H
W = 8
DIL = 2
R = 4
BLK = 128 * R
NB = S // BLK
HALO = 16
MC = 256
SUB = 128

F32 = jnp.float32
BF16 = jnp.bfloat16


def _dft_tables():
    k = np.concatenate([np.arange(0, 128, 2), np.arange(1, 128, 2)]).astype(np.float64)
    u = np.arange(128, dtype=np.float64)
    fwd = []
    for r in range(R):
        th = 2.0 * np.pi * np.outer(k + 0.5, R * u + r) / (2 * BLK)
        fwd.append(np.concatenate([np.cos(th), -np.sin(th)], axis=0))
    fwd = np.stack(fwd)
    inv = np.transpose(fwd, (0, 2, 1)) / BLK
    return fwd.astype(np.float32).astype(BF16), inv.astype(np.float32).astype(BF16)


def _radix4(e, sign):
    (ar, ai), (br, bi), (cr, ci), (dr, di) = e
    s0r, s0i, d0r, d0i = ar + cr, ai + ci, ar - cr, ai - ci
    s1r, s1i, d1r, d1i = br + dr, bi + di, br - dr, bi - di
    plus = (d0r - d1i, d0i + d1r)
    minus = (d0r + d1i, d0i - d1r)
    o1, o3 = (minus, plus) if sign < 0 else (plus, minus)
    return [(s0r + s1r, s0i + s1i), o1, (s0r - s1r, s0i - s1i), o3]


def _kernel(q_hbm, k_hbm, v_hbm, shift_ref, h_hbm, ssmd_ref, wqkv_hbm, wo_hbm, gate_ref,
            fwd_ref, inv_ref, out_hbm,
            x_s, k_s, v_s, h_s, wqkv_s, wo_s, out_s,
            wt_s, wof_s, wop_s, par_s, kf_s, kv_s, ht_s, xs_s, hs_s, z_s,
            ka_s, va_s, p_s, y_s,
            sem_x, sem_w, sem_c, sem_o):
    def lanes(c):
        return pl.ds(c * 128, 128)

    def x_copy(c):
        return pltpu.make_async_copy(q_hbm.at[0, :, lanes(c)], x_s.at[c], sem_x.at[c])

    def conv_copies(c):
        return (pltpu.make_async_copy(k_hbm.at[0, :, lanes(c)], k_s.at[c], sem_c.at[0, c]),
                pltpu.make_async_copy(v_hbm.at[0, :, lanes(c)], v_s.at[c], sem_c.at[1, c]),
                pltpu.make_async_copy(h_hbm.at[lanes(c), :], h_s.at[c], sem_c.at[2, c]))

    wqkv_copy = pltpu.make_async_copy(wqkv_hbm, wqkv_s, sem_w.at[0])
    wo_copy = pltpu.make_async_copy(wo_hbm, wo_s, sem_w.at[1])

    wqkv_copy.start()
    for c in range(NT):
        x_copy(c).start()
    for c in range(NT):
        for cp in conv_copies(c):
            cp.start()
    wo_copy.start()

    eye = (lax.broadcasted_iota(jnp.int32, (8, KS), 0)
           == lax.broadcasted_iota(jnp.int32, (8, KS), 1)).astype(BF16)
    taps = lax.dot_general(eye, shift_ref[...], (((1,), (1,)), ((), ())),
                           preferred_element_type=F32)
    ssm_d = ssmd_ref[...].astype(F32).reshape(1, D)
    gate_w = gate_ref[...].astype(F32).reshape(1, D)
    for c in range(NT):
        sl = slice(c * 128, (c + 1) * 128)
        for j in range(KS):
            par_s[c, j] = jnp.broadcast_to(taps[j:j + 1, sl], (8, 128))
        par_s[c, KS] = jnp.broadcast_to(ssm_d[:, sl], (8, 128))
        par_s[c, KS + 1] = jnp.broadcast_to(gate_w[:, sl], (8, 128))

    kf_s[pl.ds(0, 8), :] = jnp.zeros((8, 128), F32)
    ka_s[pl.ds(0, HALO), :] = jnp.zeros((HALO, 128), F32)

    wqkv_copy.wait()
    for n in range(3 * NT):
        for kk in range(NT):
            wt_s[kk, pl.ds(n * 128, 128), :] = wqkv_s[lanes(kk), lanes(n)].astype(F32).T

    for c in range(NT):
        x_copy(c).wait()

    def tile_rows(a, n):
        return jnp.broadcast_to(a[None], (n // 8, 8, 128)).reshape(n, 128)

    def phase1(c, carry):
        for cp in conv_copies(c):
            cp.wait()

        for b in range(NB):
            rows = pl.ds(b * BLK, BLK)
            kf_s[pl.ds(8 + b * BLK, BLK), :] = k_s[c, rows, :].astype(F32)
        for t in range(S // 128):
            acc = None
            for j in range(KS):
                term = kf_s[pl.ds(8 + t * 128 - j, 128), :] * tile_rows(par_s[c, j], 128)
                acc = term if acc is None else acc + term
            kv_s[pl.ds(t * 128, 128), :] = acc * v_s[c, pl.ds(t * 128, 128), :].astype(F32)
            ht_s[pl.ds(t * 128, 128), :] = h_s[c, :, pl.ds(t * 128, 128)].astype(F32).T

        def forward(src, b):
            e = []
            for r in range(R):
                dec = src[pl.ds(b * BLK + r, 128, stride=R), :].astype(BF16)
                er = jnp.dot(fwd_ref[r], dec, preferred_element_type=F32)
                e.append((er[:128], er[128:]))
            return _radix4(e, -1)

        for b in range(NB):
            for j, (re, im) in enumerate(forward(kv_s, b)):
                xs_s[b, j, 0] = re
                xs_s[b, j, 1] = im
            for j, (re, im) in enumerate(forward(ht_s, b)):
                if b == 0:
                    re = re + tile_rows(par_s[c, KS], 128)
                hs_s[b, j, 0] = re
                hs_s[b, j, 1] = im

        for g in range(128 // 16):
            rows = pl.ds(g * 16, 16)
            even = g < 4
            z = [[None] * R for _ in range(NB)]
            for j in range(R):
                xv = [(xs_s[b, j, 0, rows, :], xs_s[b, j, 1, rows, :]) for b in range(NB)]
                hv = [(hs_s[b, j, 0, rows, :], hs_s[b, j, 1, rows, :]) for b in range(NB)]
                hp = [hv[0]]
                for m in range(1, NB):
                    if even:
                        hp.append((hv[m][0] - hv[m - 1][1], hv[m][1] + hv[m - 1][0]))
                    else:
                        hp.append((hv[m][0] + hv[m - 1][1], hv[m][1] - hv[m - 1][0]))
                for i in range(NB):
                    zr = zi = None
                    for m in range(i + 1):
                        (hr, hi), (xr, xi) = hp[m], xv[i - m]
                        pr = hr * xr - hi * xi
                        pi = hr * xi + hi * xr
                        zr = pr if zr is None else zr + pr
                        zi = pi if zi is None else zi + pi
                    z[i][j] = (zr, zi)
            for i in range(NB):
                for r, (re, im) in enumerate(_radix4(z[i], +1)):
                    z_s[c, i, r, pl.ds(g * 16, 16), :] = re.astype(BF16)
                    z_s[c, i, r, pl.ds(128 + g * 16, 16), :] = im.astype(BF16)

        wc = jnp.concatenate(
            [jnp.concatenate(
                [wt_s[kk, pl.ds(part * D + 4 * c + dd, H, stride=DH), :]
                 for part in range(3) for dd in range(4)], axis=0).astype(BF16)
             for kk in range(NT)], axis=1)
        for t in range(S // MC):
            rows = pl.ds(t * MC, MC)
            xt = jnp.concatenate([x_s[kk, rows, :] for kk in range(NT)], axis=1)
            qkv = lax.dot_general(xt, wc, (((1,), (1,)), ((), ())), preferred_element_type=F32)
            ka_s[pl.ds(HALO + t * MC, MC), :] = qkv[:, 128:256]
            va_s[c, pl.ds(HALO + t * MC, MC), :] = qkv[:, 256:384]
            if t == 0:
                va_s[c, pl.ds(0, HALO), :] = jnp.broadcast_to(qkv[0:1, 256:384], (HALO, 128))
            qt = qkv[:, 0:128]
            for w in range(W):
                prod = qt * ka_s[pl.ds(HALO + t * MC - DIL * w, MC), :]
                p_s[w, rows, :] = p_s[w, rows, :] + prod
        return carry

    p_s[...] = jnp.zeros(p_s.shape, F32)
    lax.fori_loop(0, NT, phase1, 0)

    wo_copy.wait()
    for n in range(NT):
        wof_s[n] = wo_s[:, lanes(n)].astype(F32)
    for n in range(NT):
        for d in range(DH):
            wop_s[pl.ds(d * H, H), lanes(n)] = wof_s[n, pl.ds(d, H, stride=DH), :].astype(BF16)

    scale = DH ** -0.5
    row = lax.broadcasted_iota(jnp.int32, (HALO, 128), 0)
    for w in range(1, W):
        p_s[w, pl.ds(0, HALO), :] = jnp.where(row < DIL * w, -0.25e9 / scale,
                                              p_s[w, pl.ds(0, HALO), :])

    def out_copy(i):
        rows = pl.ds(pl.multiple_of(i * BLK, BLK), BLK)
        return pltpu.make_async_copy(out_s.at[rows, :], out_hbm.at[0, rows, :], sem_o.at[i])

    def phase2(i, carry):
        for c in range(NT):
            for r in range(R):
                y_s[c, pl.ds(r, 128, stride=R), :] = jnp.dot(
                    inv_ref[r], z_s[c, i, r], preferred_element_type=F32)
        for t in range(BLK // SUB):
            base = pl.multiple_of(i * BLK + t * SUB, SUB)
            rows = pl.ds(base, SUB)
            logit = []
            for w in range(W):
                a = p_s[w, rows, :]
                a = a + pltpu.roll(a, 64, 1)
                logit.append(a + pltpu.roll(a, 32, 1))
            m = logit[0]
            for w in range(1, W):
                m = jnp.maximum(m, logit[w])
            e = [jnp.exp((l - m) * scale) for l in logit]
            den = e[0]
            for w in range(1, W):
                den = den + e[w]
            inv = 1.0 / den
            o = []
            for c in range(NT):
                acc = None
                for w in range(W):
                    term = e[w] * va_s[c, pl.ds(base + (HALO - DIL * w), SUB), :]
                    acc = term if acc is None else acc + term
                o.append((acc * inv).astype(BF16))
            b = jnp.dot(jnp.concatenate(o, axis=1), wop_s[...], preferred_element_type=F32)
            xq = [x_s[c, rows, :].astype(F32) for c in range(NT)]
            gs = None
            for c in range(NT):
                term = xq[c] * tile_rows(par_s[c, KS + 1], SUB)
                gs = term if gs is None else gs + term
            g = jax.nn.sigmoid(jnp.sum(gs, axis=1, keepdims=True))
            for c in range(NT):
                a = xq[c] * y_s[c, pl.ds(t * SUB, SUB), :]
                out_s[rows, lanes(c)] = (g * a + (1.0 - g) * b[:, c * 128:(c + 1) * 128]
                                         ).astype(BF16)
        out_copy(i).start()
        return carry

    lax.fori_loop(0, NB, phase2, 0)
    for i in range(NB):
        out_copy(i).wait()


@jax.jit
def pallas_gated_mix__ssm_conv_h3__sliding_local_dilated__prompt_kernel(
    A_q: jax.Array,
    A_k: jax.Array,
    A_v: jax.Array,
    A_shift_k: jax.Array,
    A_ssm_k: jax.Array,
    A_ssm_D: jax.Array,
    B_x: jax.Array,
    B_wqkv: jax.Array,
    B_wo: jax.Array,
    gate_w: jax.Array,
):
    del B_x
    fwd, inv = _dft_tables()
    hbm = pl.BlockSpec(memory_space=pl.ANY)
    vmem = pl.BlockSpec(memory_space=pltpu.VMEM)
    scratch = [
        pltpu.VMEM((NT, S, 128), BF16),
        pltpu.VMEM((NT, S, 128), BF16),
        pltpu.VMEM((NT, S, 128), BF16),
        pltpu.VMEM((NT, 128, S), BF16),
        pltpu.VMEM((D, 3 * D), BF16),
        pltpu.VMEM((D, D), BF16),
        pltpu.VMEM((S, D), BF16),
        pltpu.VMEM((NT, 3 * D, 128), F32),
        pltpu.VMEM((NT, D, 128), F32),
        pltpu.VMEM((D, D), BF16),
        pltpu.VMEM((NT, KS + 2, 8, 128), F32),
        pltpu.VMEM((8 + S, 128), F32),
        pltpu.VMEM((S, 128), F32),
        pltpu.VMEM((S, 128), F32),
        pltpu.VMEM((NB, R, 2, 128, 128), F32),
        pltpu.VMEM((NB, R, 2, 128, 128), F32),
        pltpu.VMEM((NT, NB, R, 256, 128), BF16),
        pltpu.VMEM((HALO + S, 128), F32),
        pltpu.VMEM((NT, HALO + S, 128), F32),
        pltpu.VMEM((W, S, 128), F32),
        pltpu.VMEM((NT, BLK, 128), F32),
        pltpu.SemaphoreType.DMA((NT,)),
        pltpu.SemaphoreType.DMA((2,)),
        pltpu.SemaphoreType.DMA((3, NT)),
        pltpu.SemaphoreType.DMA((NB,)),
    ]
    return pl.pallas_call(
        _kernel,
        out_shape=jax.ShapeDtypeStruct((1, S, D), BF16),
        in_specs=[hbm, hbm, hbm, vmem, hbm, vmem, hbm, hbm, vmem, vmem, vmem],
        out_specs=hbm,
        scratch_shapes=scratch,
        compiler_params=pltpu.CompilerParams(vmem_limit_bytes=100 * 1024 * 1024),
    )(A_q, A_k, A_v, A_shift_k, A_ssm_k, A_ssm_D, B_wqkv, B_wo, gate_w, fwd, inv)
```

```python
import numpy as np
import jax
import jax.numpy as jnp
from jax import lax
from jax.experimental import pallas as pl
from jax.experimental.pallas import tpu as pltpu

S = 2048
D = 640
NT = D // 128
KS = 4
H = 32
DH = D // H
W = 8
DIL = 2
R = 4
BLK = 128 * R
NB = S // BLK
HALO = 16
MC = 128
QT = 32
HEAD = 5
SUB = 128
AT = 16
FT = 32
LOG2E = 1.4426950408889634

F32 = jnp.float32
BF16 = jnp.bfloat16
U32 = jnp.uint32


def _dft_tables():
    k = np.concatenate([np.arange(0, 128, 2), np.arange(1, 128, 2)]).astype(np.float64)
    u = np.arange(128, dtype=np.float64)
    fwd = []
    for r in range(R):
        th = 2.0 * np.pi * np.outer(k + 0.5, R * u + r) / (2 * BLK)
        fwd.append(np.stack([np.cos(th).reshape(16, 8, 128), -np.sin(th).reshape(16, 8, 128)],
                            axis=1).reshape(256, 128))
    fwd = np.stack(fwd)
    inv = fwd.reshape(R, 16, 2, 8, 128).transpose(0, 1, 3, 2, 4).reshape(R, 2, 128, 128)
    inv = np.transpose(inv, (0, 1, 3, 2)) / BLK
    return fwd.astype(np.float32).astype(BF16), inv.astype(np.float32).astype(BF16)


def _radix4(e, sign):
    (ar, ai), (br, bi), (cr, ci), (dr, di) = e
    s0r, s0i, d0r, d0i = ar + cr, ai + ci, ar - cr, ai - ci
    s1r, s1i, d1r, d1i = br + dr, bi + di, br - dr, bi - di
    plus = (d0r - d1i, d0i + d1r)
    minus = (d0r + d1i, d0i - d1r)
    o1, o3 = (minus, plus) if sign < 0 else (plus, minus)
    return [(s0r + s1r, s0i + s1i), o1, (s0r - s1r, s0i - s1i), o3]


def _interleave(*streams):
    order = sorted(((i + 0.5 * (n + 1) / len(streams)) / len(st), n, i)
                   for n, st in enumerate(streams) for i in range(len(st)))
    for _, n, i in order:
        streams[n][i]()


def _load_bf16(ref32, *idx):
    return pltpu.bitcast(ref32[idx], BF16)


def _pack(even, odd):
    return pltpu.pack_elementwise([even, odd], packed_dtype=BF16)


def _unpack(words, index):
    return pltpu.unpack_elementwise(words, index=index, packed_dtype=BF16, unpacked_dtype=F32)


def _kernel(q_hbm, k_hbm, v_hbm, shift_ref, h_hbm, ssmd_ref, wqkv_hbm, wo_hbm, gate_ref,
            fwd_hbm, inv_hbm, out_hbm,
            x_s, k_s, v_s, h_s, wqk_s, wvi_s, wo_s, out_s, fwd_s, inv_s,
            wt_s, wvt_s, wof_s, wop_s, wc_s, wv_s, par_s, kf_s, kv_s, ht_s, xs_s, hs_s, z_s,
            qa_s, ka_s, va_s, p_s, y_s, o_s, g_s,
            sem_x, sem_w, sem_c, sem_o):
    def lanes(c):
        return pl.ds(c * 128, 128)

    def x_copy(c):
        return pltpu.make_async_copy(q_hbm.at[0, :, lanes(c)], x_s.at[c], sem_x.at[c])

    def conv_copies(c):
        return (pltpu.make_async_copy(k_hbm.at[0, :, lanes(c)], k_s.at[c], sem_c.at[0, c]),
                pltpu.make_async_copy(v_hbm.at[0, :, lanes(c)], v_s.at[c], sem_c.at[1, c]),
                pltpu.make_async_copy(h_hbm.at[lanes(c), :], h_s.at[c], sem_c.at[2, c]),
                pltpu.make_async_copy(wqkv_hbm.at[lanes(c), pl.ds(2 * D, D)], wvi_s.at[c],
                                      sem_c.at[3, c]),
                pltpu.make_async_copy(wo_hbm.at[:, lanes(c)], wo_s.at[c], sem_c.at[4, c]))

    def w_copy(kk):
        return pltpu.make_async_copy(wqkv_hbm.at[lanes(kk), pl.ds(0, 2 * D)], wqk_s.at[kk],
                                     sem_w.at[kk])

    fwd_copy = pltpu.make_async_copy(fwd_hbm, fwd_s, sem_w.at[NT])
    inv_copy = pltpu.make_async_copy(inv_hbm, inv_s, sem_w.at[NT + 1])

    queue = ([w_copy(kk) for kk in range(NT)] + [x_copy(c) for c in range(NT)]
             + [fwd_copy] + list(conv_copies(0)))
    ahead = 3
    for cp in queue[:ahead]:
        cp.start()

    x32 = x_s.bitcast(U32)
    fwd32 = fwd_s.bitcast(U32)
    inv32 = inv_s.bitcast(U32)

    taps = shift_ref[...].astype(F32)
    ssm_d = ssmd_ref[...].astype(F32).reshape(1, D)
    gate_w = gate_ref[...].astype(F32).reshape(1, D)
    for c in range(NT):
        sl = slice(c * 128, (c + 1) * 128)
        for j in range(KS):
            par_s[c, j] = jnp.broadcast_to(taps[j:j + 1, sl], (8, 128))
        par_s[c, KS] = jnp.broadcast_to(ssm_d[:, sl], (8, 128))
        par_s[c, KS + 1] = jnp.broadcast_to(gate_w[:, sl], (8, 128))

    kf_s[pl.ds(0, 8), :] = jnp.zeros((8, 128), F32)
    ka_s[pl.ds(0, HALO), :] = jnp.zeros((HALO, 128), F32)

    for pos in range(2 * NT):
        queue[pos].wait()
        if pos + ahead < len(queue):
            queue[pos + ahead].start()
        if pos < NT:
            for n in range(2 * NT):
                wt_s[pos, lanes(n), :] = wqk_s[pos, :, lanes(n)].astype(F32).T
        elif pos < NT + 4:
            for w in range(2):
                p_s[2 * (pos - NT) + w] = jnp.zeros((S, 128), F32)
    for cp in queue[2 * NT + ahead:]:
        cp.start()
    fwd_copy.wait()

    def tile_rows(a, n):
        return jnp.broadcast_to(a[None], (n // 8, 8, 128)).reshape(n, 128)

    def head_rows(ref, start):
        return _pack(ref[pl.ds(start, H // 2, stride=2 * DH), :],
                     ref[pl.ds(start + DH, H // 2, stride=2 * DH), :])

    scale = DH ** -0.5

    def phase1(c, carry):
        def conv_wait():
            for cp in conv_copies(c):
                cp.wait()

            @pl.when(c + 1 < NT)
            def _():
                for cp in conv_copies(c + 1):
                    cp.start()

            @pl.when(c + 1 == NT)
            def _():
                inv_copy.start()

        def conv_in(t):
            def run():
                rows = pl.ds(t * 128, 128)
                kf_s[pl.ds(8 + t * 128, 128), :] = k_s[c, rows, :].astype(F32)
                acc = None
                for j in range(KS):
                    term = kf_s[pl.ds(8 + t * 128 - j, 128), :] * tile_rows(par_s[c, j], 128)
                    acc = term if acc is None else acc + term
                kv_s[rows, :] = acc * v_s[c, rows, :].astype(F32)
                ht_s[pl.ds(t * 64, 64), :] = pltpu.bitcast(h_s[c, :, rows].T, U32)
            return run

        def kv_samples(b, r):
            return kv_s[pl.ds(b * BLK + r, 128, stride=R), :]

        def h_samples(b, r):
            return _unpack(ht_s[pl.ds(b * BLK // 2 + r // 2, 128, stride=R // 2), :], r % 2)

        def forward(src, dst, b, skip_term):
            def run():
                e = []
                for r in range(R):
                    e.append(jnp.dot(_load_bf16(fwd32, r), src(b, r).astype(BF16),
                                     preferred_element_type=F32))
                for g in range(16):
                    lo, hi = slice(g * 16, g * 16 + 8), slice(g * 16 + 8, g * 16 + 16)
                    for j, (re, im) in enumerate(_radix4([(er[lo], er[hi]) for er in e], -1)):
                        if skip_term:
                            re = re + par_s[c, KS]
                        dst[b, j, lo, :] = re
                        dst[b, j, hi, :] = im
            return run

        def pointwise(g):
            def run():
                lo, hi = pl.ds(g * 16, 8), pl.ds(g * 16 + 8, 8)
                even = g < 8
                z = [[None] * R for _ in range(NB)]
                for j in range(R):
                    xv = [(xs_s[b, j, lo, :], xs_s[b, j, hi, :]) for b in range(NB)]
                    hv = [(hs_s[b, j, lo, :], hs_s[b, j, hi, :]) for b in range(NB)]
                    hp = [hv[0]]
                    for m in range(1, NB):
                        if even:
                            hp.append((hv[m][0] - hv[m - 1][1], hv[m][1] + hv[m - 1][0]))
                        else:
                            hp.append((hv[m][0] + hv[m - 1][1], hv[m][1] - hv[m - 1][0]))
                    for i in range(NB):
                        zr = zi = None
                        for m in range(i + 1):
                            (hr, hi_), (xr, xi) = hp[m], xv[i - m]
                            pr = hr * xr - hi_ * xi
                            pi = hr * xi + hi_ * xr
                            zr = pr if zr is None else zr + pr
                            zi = pi if zi is None else zi + pi
                        z[i][j] = (zr, zi)
                for i in range(NB):
                    for r, (re, im) in enumerate(_radix4(z[i], +1)):
                        z_s[c, i, r, pl.ds(g * 8, 8), :] = _pack(re, im)
            return run

        def weights():
            for kk in range(NT):
                for part in range(2):
                    for dd in range(4):
                        wc_s[kk, pl.ds(part * 64 + dd * 16, 16), :] = head_rows(
                            wt_s.at[kk], part * D + 4 * c + dd)

        def late_weights():
            for n in range(NT):
                wvt_s[lanes(n), :] = wvi_s[c, :, lanes(n)].astype(F32).T
            wof_s[...] = wo_s[c].astype(F32)
            for d in range(DH):
                wv_s[c, pl.ds(d * 16, 16), :] = head_rows(wvt_s, d)
                wop_s[c, pl.ds(d * 16, 16), :] = head_rows(wof_s, d)

        def project(t):
            def run():
                xt = jnp.concatenate([_load_bf16(x32, kk, pl.ds(t * MC // 2, MC // 2))
                                      for kk in range(NT)], axis=1)
                wc = jnp.concatenate([_load_bf16(wc_s, kk) for kk in range(NT)], axis=1)
                qkv = lax.dot_general(xt, wc, (((1,), (1,)), ((), ())),
                                      preferred_element_type=F32)
                qa_s[pl.ds(t * MC, MC), :] = qkv[:, 0:128] * (scale * LOG2E)
                ka_s[pl.ds(HALO + t * MC, MC), :] = qkv[:, 128:256]
            return run

        def logits(t):
            def run():
                for u in range(t * MC, (t + 1) * MC, QT):
                    rows = pl.ds(u, QT)
                    qt = qa_s[rows, :]
                    for w in range(W):
                        prod = qt * ka_s[pl.ds(HALO + u - DIL * w, QT), :]
                        p_s[w, rows, :] = p_s[w, rows, :] + prod
            return run

        n_mc = S // MC
        proj = [project(t) for t in range(n_mc)]
        attn = [proj[0]]
        for t in range(1, n_mc):
            attn += [proj[t], logits(t - 1)]
        attn.append(logits(n_mc - 1))
        conv = []
        for b in range(NB):
            conv += [conv_in(4 * b + u) for u in range(4)]
            conv += [forward(kv_samples, xs_s, b, False), forward(h_samples, hs_s, b, b == 0)]
        conv += [pointwise(g) for g in range(16)] + [late_weights]
        weights()
        for f in attn[:HEAD]:
            f()
        conv_wait()
        _interleave(attn[HEAD:], conv)

        return carry

    lax.fori_loop(0, NT, phase1, 0)
    inv_copy.wait()

    row = lax.broadcasted_iota(jnp.int32, (HALO, 128), 0)
    for w in range(1, W):
        p_s[w, pl.ds(0, HALO), :] = jnp.where(row < DIL * w, -0.25e9 * LOG2E,
                                              p_s[w, pl.ds(0, HALO), :])

    def out_copy(i):
        rows = pl.ds(i * SUB, SUB)
        return pltpu.make_async_copy(out_s.at[rows, :], out_hbm.at[0, rows, :], sem_o.at[i])

    def inverse(i, c):
        def run():
            for r in range(R):
                y_s[c, pl.ds(i * BLK + r, 128, stride=R), :] = jnp.dot(
                    jnp.concatenate([_load_bf16(inv32, r, 0), _load_bf16(inv32, r, 1)], axis=1),
                    _load_bf16(z_s, c, i, r), preferred_element_type=F32)
        return run

    def values(t):
        def run():
            xt = jnp.concatenate([_load_bf16(x32, kk, pl.ds(t * SUB // 2, SUB // 2))
                                  for kk in range(NT)], axis=1)
            wv = jnp.concatenate([_load_bf16(wv_s, kk) for kk in range(NT)], axis=1)
            v = lax.dot_general(xt, wv, (((1,), (1,)), ((), ())), preferred_element_type=F32)
            for c in range(NT):
                vc = v[:, c * 128:(c + 1) * 128]
                va_s[c, pl.ds(HALO + t * SUB, SUB), :] = vc
                if t == 0:
                    va_s[c, pl.ds(0, HALO), :] = jnp.broadcast_to(vc[0:1], (HALO, 128))
        return run

    def attend(u):
        def run():
            half = []
            for par in range(2):
                rows = pl.ds(u + par, AT // 2, stride=2)
                logit = []
                for w in range(W):
                    a = p_s[w, rows, :]
                    a = a + pltpu.roll(a, 64, 1)
                    logit.append(a + pltpu.roll(a, 32, 1))
                m = logit[0]
                for w in range(1, W):
                    m = jnp.maximum(m, logit[w])
                e = [jnp.exp2(l - m) for l in logit]
                den = e[0]
                for w in range(1, W):
                    den = den + e[w]
                inv = pl.reciprocal(den, approx=True)
                inv = inv * (2.0 - den * inv)
                gs = None
                for c in range(NT):
                    term = _unpack(x32[c, pl.ds(u // 2, AT // 2), :], par) * tile_rows(
                        par_s[c, KS + 1], AT // 2)
                    gs = term if gs is None else gs + term
                th = 0.5 * jnp.tanh(0.5 * jnp.sum(gs, axis=1, keepdims=True))
                g_s[rows, :] = jnp.broadcast_to(0.5 + th, (AT // 2, 128))
                inv = inv * (0.5 - th)
                acc = []
                for c in range(NT):
                    a = None
                    for w in range(W):
                        term = e[w] * va_s[c, pl.ds(u + par + HALO - DIL * w, AT // 2, stride=2), :]
                        a = term if a is None else a + term
                    acc.append(a * inv)
                half.append(acc)
            for c in range(NT):
                o_s[c, pl.ds(u // 2, AT // 2), :] = _pack(half[0][c], half[1][c])
        return run

    def finish(t):
        def run():
            half = pl.ds(t * SUB // 2, SUB // 2)
            o = jnp.concatenate([_load_bf16(o_s, c, half) for c in range(NT)], axis=1)
            wo = jnp.concatenate([_load_bf16(wop_s, n) for n in range(NT)], axis=1)
            b = jnp.dot(o, wo, preferred_element_type=F32)
            for u in range(0, SUB, FT):
                rws = pl.ds(t * SUB + u, FT)
                g = g_s[rws, :]
                for c in range(NT):
                    a = x_s[c, rws, :].astype(F32) * y_s[c, rws, :]
                    out_s[rws, lanes(c)] = (
                        g * a + b[u:u + FT, c * 128:(c + 1) * 128]).astype(BF16)
            out_copy(t).start()
        return run

    n_sub = S // SUB
    per = SUB // AT
    att = [attend(u) for u in range(0, S, AT)]
    inv_tasks = [[inverse(i, c) for c in range(NT)] for i in range(NB)]
    values(0)()
    values(1)()
    _interleave(inv_tasks[0], att[:per])
    for t in range(n_sub):
        i, sub = divmod(t, BLK // SUB)
        mxu = [finish(t)]
        if t + 2 < n_sub:
            mxu.append(values(t + 2))
        if i + 1 < NB:
            n = BLK // SUB
            mxu += inv_tasks[i + 1][sub * NT // n:(sub + 1) * NT // n]
        _interleave(mxu, att[(t + 1) * per:(t + 2) * per])
    for t in range(n_sub):
        out_copy(t).wait()


@jax.jit
def pallas_gated_mix__ssm_conv_h3__sliding_local_dilated__prompt_kernel(
    A_q: jax.Array,
    A_k: jax.Array,
    A_v: jax.Array,
    A_shift_k: jax.Array,
    A_ssm_k: jax.Array,
    A_ssm_D: jax.Array,
    B_x: jax.Array,
    B_wqkv: jax.Array,
    B_wo: jax.Array,
    gate_w: jax.Array,
):
    del B_x
    fwd, inv = _dft_tables()
    hbm = pl.BlockSpec(memory_space=pl.ANY)
    vmem = pl.BlockSpec(memory_space=pltpu.VMEM)
    scratch = [
        pltpu.VMEM((NT, S, 128), BF16),
        pltpu.VMEM((NT, S, 128), BF16),
        pltpu.VMEM((NT, S, 128), BF16),
        pltpu.VMEM((NT, 128, S), BF16),
        pltpu.VMEM((NT, 128, 2 * D), BF16),
        pltpu.VMEM((NT, 128, D), BF16),
        pltpu.VMEM((NT, D, 128), BF16),
        pltpu.VMEM((S, D), BF16),
        pltpu.VMEM((R, 256, 128), BF16),
        pltpu.VMEM((R, 2, 128, 128), BF16),
        pltpu.VMEM((NT, 2 * D, 128), F32),
        pltpu.VMEM((D, 128), F32),
        pltpu.VMEM((D, 128), F32),
        pltpu.VMEM((NT, D // 2, 128), U32),
        pltpu.VMEM((NT, 128, 128), U32),
        pltpu.VMEM((NT, D // 2, 128), U32),
        pltpu.VMEM((NT, KS + 2, 8, 128), F32),
        pltpu.VMEM((8 + S, 128), F32),
        pltpu.VMEM((S, 128), F32),
        pltpu.VMEM((S // 2, 128), U32),
        pltpu.VMEM((NB, R, 256, 128), F32),
        pltpu.VMEM((NB, R, 256, 128), F32),
        pltpu.VMEM((NT, NB, R, 128, 128), U32),
        pltpu.VMEM((S, 128), F32),
        pltpu.VMEM((HALO + S, 128), F32),
        pltpu.VMEM((NT, HALO + S, 128), F32),
        pltpu.VMEM((W, S, 128), F32),
        pltpu.VMEM((NT, S, 128), F32),
        pltpu.VMEM((NT, S // 2, 128), U32),
        pltpu.VMEM((S, 128), F32),
        pltpu.SemaphoreType.DMA((NT,)),
        pltpu.SemaphoreType.DMA((NT + 2,)),
        pltpu.SemaphoreType.DMA((5, NT)),
        pltpu.SemaphoreType.DMA((S // SUB,)),
    ]
    return pl.pallas_call(
        _kernel,
        out_shape=jax.ShapeDtypeStruct((1, S, D), BF16),
        in_specs=[hbm, hbm, hbm, vmem, hbm, vmem, hbm, hbm, vmem, hbm, hbm],
        out_specs=hbm,
        scratch_shapes=scratch,
        compiler_params=pltpu.CompilerParams(vmem_limit_bytes=100 * 1024 * 1024),
    )(A_q, A_k, A_v, A_shift_k.T, A_ssm_k, A_ssm_D, B_wqkv, B_wo, gate_w, fwd, inv)
```

```python
import numpy as np
import jax
import jax.numpy as jnp
from jax import lax
from jax.experimental import pallas as pl
from jax.experimental.pallas import tpu as pltpu

S = 2048
D = 640
NT = D // 128
KS = 4
H = 32
DH = D // H
W = 8
DIL = 2
R = 4
BLK = 128 * R
NB = S // BLK
HALO = 16
P0 = 416
HEAD_CHUNKS = ((0, 128), (128, 144), (272, 144))
P1 = 192
RS = (S - P0 - P1) // NT
CHUNKS = ((0, 144), (144, 144))
LAG = 144
PAD = 16
QT = 16
HEAD = 4
GAP = 2
EARLY = 3
REST = 250
PACE = ("kv", "q")
ZST = 1
ST = 16
TILES = ((0, 1, 2), (3, 4))
GATE_Y = True
IDLE = 100
FM = 128
SUB = 128
AT = 16
FT = 32
LEAD = 3
SLACK = 900
FLAGS = None
LOG2E = 1.4426950408889634

F32 = jnp.float32
BF16 = jnp.bfloat16
U32 = jnp.uint32


def _dft_tables():
    k = np.concatenate([np.arange(0, 128, 2), np.arange(1, 128, 2)]).astype(np.float64)
    u = np.arange(128, dtype=np.float64)
    fwd = []
    for r in range(R):
        th = 2.0 * np.pi * np.outer(k + 0.5, R * u + r) / (2 * BLK)
        fwd.append(np.stack([np.cos(th).reshape(16, 8, 128), -np.sin(th).reshape(16, 8, 128)],
                            axis=1).reshape(256, 128))
    fwd = np.stack(fwd)
    fwd_in = fwd.reshape(R, 256, 8, 2, 8).transpose(0, 1, 2, 4, 3).reshape(R, 256, 128)
    inv = fwd.reshape(R, 16, 2, 8, 128).transpose(0, 1, 3, 2, 4).reshape(R, 2, 128, 128)
    inv = np.transpose(inv, (0, 1, 3, 2)) / BLK
    return fwd_in.astype(np.float32).astype(BF16), inv.astype(np.float32).astype(BF16)


def _radix4(e, sign):
    (ar, ai), (br, bi), (cr, ci), (dr, di) = e
    s0r, s0i, d0r, d0i = ar + cr, ai + ci, ar - cr, ai - ci
    s1r, s1i, d1r, d1i = br + dr, bi + di, br - dr, bi - di
    plus = (d0r - d1i, d0i + d1r)
    minus = (d0r + d1i, d0i - d1r)
    o1, o3 = (minus, plus) if sign < 0 else (plus, minus)
    return [(s0r + s1r, s0i + s1i), o1, (s0r - s1r, s0i - s1i), o3]


def _interleave(*streams):
    todo = [list(st) for st in streams]
    total = [sum(t[1] for t in st) or 1 for st in streams]
    names = {t[0] for st in streams for t in st}
    spent = [0] * len(streams)
    done = set()
    while any(todo):
        ready = [n for n, st in enumerate(todo)
                 if st and all(d in done or d not in names for d in st[0][2])]
        n = min(ready, key=lambda n: (spent[n] + 0.5 * todo[n][0][1]) / total[n])
        name, cost, _, run = todo[n].pop(0)
        run()
        spent[n] += cost
        done.add(name)


def _load_bf16(ref32, *idx):
    return pltpu.bitcast(ref32[idx], BF16)


def _pack(even, odd):
    return pltpu.pack_elementwise([even, odd], packed_dtype=BF16)


def _unpack(words, index):
    return pltpu.unpack_elementwise(words, index=index, packed_dtype=BF16, unpacked_dtype=F32)


def _kernel(q_hbm, k_hbm, v_hbm, shift_ref, h_hbm, ssmd_ref, wqkv_hbm, wo_hbm, gate_ref,
            fwd_hbm, inv_hbm, zero_ref, out_hbm,
            x_s, kv_s, h_s, wqk_s, wvi_s, wo_s, out_s, fwd_s, inv_s,
            wt_s, wop_s, wc_s, wv_s, par_s, ht_s, dec_s, spec0_s, spec1_s, f_s,
            qa_s, ka_s, p_s, pw_s, va_s, y_s, o_s,
            sem_x, sem_w, sem_c, sem_o):
    spec_s = (spec0_s, spec1_s)

    def lanes(c):
        return pl.ds(c * 128, 128)

    def x_copies(start, size, sem):
        rows = pl.ds(start, size)
        return [pltpu.make_async_copy(q_hbm.at[0, rows, lanes(kk)], x_s.at[kk, rows], sem)
                for kk in range(NT)]

    def step_copies(c):
        start = P0 + c * RS
        cps = [(h_hbm.at[lanes(c), :], h_s.at[c]),
               (k_hbm.at[0, :, lanes(c)], kv_s.at[c, pl.ds(PAD, S)]),
               (v_hbm.at[0, :, lanes(c)], kv_s.at[NT + c, pl.ds(0, S)]),
               (wqkv_hbm.at[lanes(c), pl.ds(2 * D, D)], wvi_s.at[c]),
               (wo_hbm.at[:, lanes(c)], wo_s.at[c])]
        return (x_copies(start, RS, sem_c.at[c])
                + [pltpu.make_async_copy(src, dst, sem_c.at[c]) for src, dst in cps])

    def w_copy(n):
        kk, part = divmod(n, 2)
        cols = pl.ds(part * D, D)
        return pltpu.make_async_copy(wqkv_hbm.at[lanes(kk), cols], wqk_s.at[kk, :, cols],
                                     sem_w.at[n])

    fwd_copy = pltpu.make_async_copy(fwd_hbm, fwd_s, sem_w.at[2 * NT])
    last_copies = [pltpu.make_async_copy(inv_hbm, inv_s, sem_w.at[2 * NT + 1])]
    if P1:
        last_copies += x_copies(S - P1, P1, sem_w.at[2 * NT + 1])

    head_x = [x_copies(start, size, sem_x.at[n]) for n, (start, size) in enumerate(HEAD_CHUNKS)]
    for cp in (head_x[0] + [w_copy(n) for n in range(2 * NT)] + sum(head_x[1:], [])
               + [fwd_copy] + step_copies(0)):
        cp.start()

    zero, zero_st, zero_pace = zero_ref[0], zero_ref[ZST], zero_ref[2]

    def spectra(c):
        return spec_s[c % 2].at[zero], spec_s[c % 2].at[zero + 1]

    def z_of(c):
        return spec_s[c % 2].at[zero_st + 2 + c // 2]

    x32 = x_s.bitcast(U32)
    kv32 = kv_s.bitcast(U32)

    paced = []

    def pace(result):
        for name in paced:
            if name == "kv":
                kv32[zero_pace + 2 * NT, pl.ds(S // 2, 8), :] = pltpu.bitcast(result[:8], U32)
            elif name == "q":
                qa_s[zero_pace, pl.ds(S, 8), :] = result[:8]
            else:
                spec_s[name][zero_pace + 5, 0, 0, pl.ds(0, 8), :] = result[:8]
    fwd32 = fwd_s.bitcast(U32)
    inv32 = inv_s.bitcast(U32)

    taps = shift_ref[...].astype(F32)
    ssm_d = ssmd_ref[...].astype(F32).reshape(1, D)
    gate_w = gate_ref[...].astype(F32).reshape(1, D)
    for c in range(NT):
        sl = slice(c * 128, (c + 1) * 128)
        for j in range(KS):
            par_s[c, j] = jnp.broadcast_to(taps[j:j + 1, sl], (8, 128))
        par_s[c, KS] = jnp.broadcast_to(ssm_d[:, sl], (8, 128))
        par_s[c, KS + 1] = jnp.broadcast_to(gate_w[:, sl], (8, 128))

    for c in range(NT):
        ka_s[c, pl.ds(0, HALO), :] = jnp.zeros((HALO, 128), F32)
        kv_s[c, pl.ds(0, PAD), :] = jnp.zeros((PAD, 128), BF16)

    def tile_rows(a, n):
        return jnp.broadcast_to(a[None], (n // 8, 8, 128)).reshape(n, 128)

    def head_rows(ref, start):
        return _pack(ref[pl.ds(start, H // 2, stride=2 * DH), :],
                     ref[pl.ds(start + DH, H // 2, stride=2 * DH), :])

    scale = DH ** -0.5

    for n in range(2 * NT):
        kk, part = divmod(n, 2)
        w_copy(n).wait()
        for j in range(NT):
            wt_s[n % 2, lanes(j), :] = wqk_s[kk, :, lanes(part * NT + j)].astype(F32).T
        for d in range(DH):
            wc_s[kk, pl.ds(part * D // 2 + d * 16, 16), :] = head_rows(wt_s.at[n % 2], d)

    def project(base, size, which, n):
        def run():
            xt = jnp.concatenate([_load_bf16(x32, kk, pl.ds(base // 2, size // 2))
                                  for kk in range(NT)], axis=1)
            wc = jnp.concatenate([_load_bf16(wc_s, kk, pl.ds(which * D // 2 + n * 64, 64))
                                  for kk in range(NT)], axis=1)
            res = lax.dot_general(xt, wc, (((1,), (1,)), ((), ())), preferred_element_type=F32)
            if which == 0:
                qa_s[n, pl.ds(base, size), :] = res
            else:
                ka_s[n, pl.ds(base + HALO, size), :] = res
            pace(res)
        return run

    def logits(base):
        def run():
            qt = [qa_s[n, pl.ds(base, QT), :] for n in range(NT)]
            for w in range(W):
                acc = None
                for n in range(NT):
                    term = qt[n] * ka_s[n, pl.ds(base + (HALO - DIL * w), QT), :]
                    acc = term if acc is None else acc + term
                p_s[w, pl.ds(base, QT), :] = acc
        return run

    def project_tasks(tag, base, size):
        return [(("proj", tag, which, n), size * 5 // 4, (), project(base, size, which, n))
                for which in (1, 0) for n in range(NT)]

    def logit_tasks(tag, base, size):
        return [(("logit", tag, u), 5 * QT // 2, (("proj", tag, 0, NT - 1),), logits(base + u))
                for u in range(0, size, QT)]

    def pointwise(z_s, xs_s, hs_s, g, j):
        def run():
            lo, hi = pl.ds(g * 16, 8), pl.ds(g * 16 + 8, 8)
            xv = [(xs_s[b, j, lo, :], xs_s[b, j, hi, :]) for b in range(NB)]
            hv = [(hs_s[b, j, lo, :], hs_s[b, j, hi, :]) for b in range(NB)]
            hp = [hv[0]]
            for m in range(1, NB):
                if g < 8:
                    hp.append((hv[m][0] - hv[m - 1][1], hv[m][1] + hv[m - 1][0]))
                else:
                    hp.append((hv[m][0] + hv[m - 1][1], hv[m][1] - hv[m - 1][0]))
            for i in range(NB):
                zr = zi = None
                for m in range(i + 1):
                    (hr, hi_), (xr, xi) = hp[m], xv[i - m]
                    pr = hr * xr - hi_ * xi
                    pi = hr * xi + hi_ * xr
                    zr = pr if zr is None else zr + pr
                    zi = pi if zi is None else zi + pi
                z_s[i, j, lo, :] = zr
                z_s[i, j, hi, :] = zi
        return run

    def pointwise_tasks(c):
        return [(("point", g, j), 21, (), pointwise(z_of(c), *spectra(c), g, j))
                for g in range(16) for j in range(R)]

    def tile_step(c):
        base = P0 + c * RS

        def next_inputs():
            for cp in (step_copies(c + 1) if c + 1 < NT else last_copies):
                cp.wait()

        def kv_samples(b, a):
            def run():
                halves = []
                for u in (b * 128 + a * 16, b * 128 + a * 16 + 8):
                    def words(slab, off):
                        return kv32[zero + slab, pl.ds(2 * u + off, 8, stride=2), :]
                    kw = {o: words(c, PAD // 2 + o) for o in (-2, -1, 0, 1)}
                    kt = {t: _unpack(kw[t // 2], t % 2) for t in range(1 - KS, R)}
                    vw = [words(NT + c, o) for o in range(R // 2)]
                    out = []
                    for r in range(R):
                        acc = None
                        for j in range(KS):
                            term = kt[r - j] * par_s[c, j]
                            acc = term if acc is None else acc + term
                        out.append(acc * _unpack(vw[r // 2], r % 2))
                    halves.append(out)
                for r in range(R):
                    kv32[2 * NT, pl.ds((b * R + r) * 64 + a * 8, 8), :] = _pack(
                        halves[0][r], halves[1][r])
            return run

        def h_transpose(t):
            def run():
                ht_s[pl.ds(t * 64, 64), :] = pltpu.bitcast(h_s[c, :, pl.ds(t * 128, 128)].T, U32)
            return run

        def h_samples(b):
            def run():
                for a in range(8):
                    for o in range(R // 2):
                        w0, w1 = (ht_s[pl.ds(2 * (b * 128 + a * 16 + e) + o, 8, stride=2), :]
                                  for e in (0, 8))
                        for e in range(2):
                            dec_s[b, 2 * o + e, pl.ds(a * 8, 8), :] = _pack(
                                _unpack(w0, e), _unpack(w1, e))
            return run

        def forward(slot, dst, b, m):
            def run():
                e = [jnp.dot(_load_bf16(fwd32, r, pl.ds(m * FM // 2, FM // 2)),
                             _load_bf16(dec_s, b, r) if slot else
                             _load_bf16(kv32, 2 * NT, pl.ds((b * R + r) * 64, 64)),
                             preferred_element_type=F32)
                     for r in range(R)]
                for g in range(FM // 16):
                    lo, hi = slice(g * 16, g * 16 + 8), slice(g * 16 + 8, g * 16 + 16)
                    for j, (re, im) in enumerate(_radix4([(er[lo], er[hi]) for er in e], -1)):
                        if slot == 1 and b == 0:
                            re = re + par_s[c, KS]
                        dst[b, j, pl.ds(m * FM + g * 16, 8), :] = re
                        dst[b, j, pl.ds(m * FM + g * 16 + 8, 8), :] = im
                pace(e[-1])
            return run

        def late_weights():
            for n in range(NT):
                wt_s[0, lanes(n), :] = wvi_s[c, :, lanes(n)].astype(F32).T
            wt_s[1] = wo_s[c].astype(F32)
            for d in range(DH):
                wv_s[c, pl.ds(d * 16, 16), :] = head_rows(wt_s.at[0], d)
                wop_s[c, pl.ds(d * 16, 16), :] = head_rows(wt_s.at[1], d)

        proj = sum((project_tasks(n, base + start, size)
                    for n, (start, size) in enumerate(CHUNKS)), [])
        point = pointwise_tasks(c - 1) if c else []
        point.append((("rest",), REST, (), lambda: None))
        xs_s, hs_s = spectra(c)
        logit = logit_tasks(-1, base - LAG, LAG)
        for n, (start, size) in enumerate(CHUNKS):
            logit += logit_tasks(n, base + start, min(size, RS - LAG - start))
        mxu, prep = proj[:HEAD], []
        for b in range(NB):
            prep += [(("ht", t), 10, (), h_transpose(t)) for t in range(4 * b, 4 * b + 4)]
            prep += [(("dec", 1, b), 24, (), h_samples(b))]
            prep += [(("dec", 0, b, a), 24, (), kv_samples(b, a)) for a in range(8)]
            for slot, dst, need in ((1, hs_s, ("dec", 1, b)), (0, xs_s, ("dec", 0, b, 7))):
                mxu += [(("fwd", slot, b, m), FM, (need,), forward(slot, dst, b, m))
                        for m in range(256 // FM)]
                lo = HEAD + (2 * b + 1 - slot) * GAP
                mxu += proj[lo:lo + GAP]
        mxu += proj[HEAD + 2 * NB * GAP:]
        mxu.insert(len(mxu) - EARLY, (("wait",), 0, (("point", 15, R - 1),), next_inputs))
        prep += [(("late",), 150, (), late_weights), (("idle",), IDLE, (), lambda: None)]
        paced[:] = [name for name in ("kv", "q", (c + 1) % 2) if name in PACE or name in (0, 1)]
        _interleave(mxu, prep, point, logit)

    done = 0
    for n, (start, size) in enumerate(HEAD_CHUNKS):
        for cp in head_x[n]:
            cp.wait()
        for c in range(1, NT):
            if (c - 1) * len(HEAD_CHUNKS) // (NT - 1) == n:
                for cp in step_copies(c):
                    cp.start()
        ready = min(start, P0 - LAG)
        _interleave(project_tasks(n, start, size), logit_tasks(-1, done, ready - done))
        done = ready
    _interleave(logit_tasks(-1, done, P0 - LAG - done))
    fwd_copy.wait()
    for cp in last_copies:
        cp.start()
    for cp in step_copies(0):
        cp.wait()
    for c in range(NT):
        tile_step(c)
    if P1:
        paced[:] = [(NT - 1) % 2, "q"]
        _interleave(project_tasks(0, S - P1, P1), pointwise_tasks(NT - 1),
                    logit_tasks(-1, S - P1 - LAG, LAG))

    row = lax.broadcasted_iota(jnp.int32, (HALO, 128), 0)
    for w in range(1, W):
        p_s[w, pl.ds(0, HALO), :] = jnp.where(row < DIL * w, -0.25e9 / scale,
                                              p_s[w, pl.ds(0, HALO), :])

    def out_copy(i):
        rows = pl.ds(i * SUB, SUB)
        return pltpu.make_async_copy(out_s.at[rows, :], out_hbm.at[0, rows, :], sem_o.at[i])

    def inverse(i, c, r):
        def run():
            y = jnp.dot(
                jnp.concatenate([_load_bf16(inv32, r, 0), _load_bf16(inv32, r, 1)], axis=1),
                _load_bf16(f_s, c, i % 2, r), preferred_element_type=F32)
            y_s[c, pl.ds(i * BLK + r, 128, stride=R), :] = y
            pace(y)
        return run

    def inverse_butterfly(i, c, part):
        def run():
            z_s = z_of(c)
            for g in range(4 * part, 4 * part + 4):
                z = [(z_s[i, j, pl.ds(g * 16, 8), :], z_s[i, j, pl.ds(g * 16 + 8, 8), :])
                     for j in range(R)]
                for r, (re, im) in enumerate(_radix4(z, +1)):
                    f_s[c, i % 2, r, pl.ds(g * 8, 8), :] = _pack(re, im)
        return run

    def values(t, n):
        def run():
            xt = jnp.concatenate([_load_bf16(x32, kk, pl.ds(t * SUB // 2, SUB // 2))
                                  for kk in range(NT)], axis=1)
            wv = jnp.concatenate([_load_bf16(wv_s, kk, pl.ds(n * 64, 64)) for kk in range(NT)],
                                 axis=1)
            v = lax.dot_general(xt, wv, (((1,), (1,)), ((), ())), preferred_element_type=F32)
            va_s[n, pl.ds(HALO + t * SUB, SUB), :] = v
            pace(v)
            if t == 0:
                va_s[n, pl.ds(0, HALO), :] = jnp.broadcast_to(v[0:1], (HALO, 128))
        return run

    def softmax(u):
        def run():
            rows = pl.ds(u, ST)
            logit = []
            for w in range(W):
                a = p_s[w, rows, :]
                a = a + pltpu.roll(a, 64, 1)
                logit.append(a + pltpu.roll(a, 32, 1))
            m = logit[0]
            for w in range(1, W):
                m = jnp.maximum(m, logit[w])
            e = [jnp.exp2((l - m) * (scale * LOG2E)) for l in logit]
            den = e[0]
            for w in range(1, W):
                den = den + e[w]
            inv = pl.reciprocal(den, approx=True)
            inv = inv * (2.0 - den * inv)
            gs = None
            for c in range(NT):
                term = x_s[c, rows, :].astype(F32) * tile_rows(par_s[c, KS + 1], ST)
                gs = term if gs is None else gs + term
            th = 0.5 * jnp.tanh(0.5 * jnp.sum(gs, axis=1, keepdims=True))
            y_s[NT, rows, :] = jnp.broadcast_to(0.5 + th, (ST, 128))
            inv = inv * (0.5 - th)
            for w in range(W):
                pw_s[w, rows, :] = e[w] * inv
        return run

    def attend(u, tiles):
        def run():
            for c in tiles:
                half = []
                for par in range(2):
                    a = None
                    for w in range(W):
                        term = (pw_s[w, pl.ds(u + par, AT // 2, stride=2), :]
                                * va_s[c, pl.ds(u + par + HALO - DIL * w, AT // 2, stride=2), :])
                        a = term if a is None else a + term
                    half.append(a)
                o_s[c, pl.ds(u // 2, AT // 2), :] = _pack(*half)
        return run

    def finish(t, n):
        def run():
            half = pl.ds(t * SUB // 2, SUB // 2)
            o = jnp.concatenate([_load_bf16(o_s, c, half) for c in range(NT)], axis=1)
            b = jnp.dot(o, _load_bf16(wop_s, n), preferred_element_type=F32)
            pace(b)
            if GATE_Y:
                y_s[zero_pace, pl.ds(S, 8), :] = b[:8]
            for u in range(0, SUB, FT):
                rws = pl.ds(t * SUB + u, FT)
                a = x_s[n, rws, :].astype(F32) * y_s[n, rws, :]
                out_s[rws, lanes(n)] = (y_s[NT, rws, :] * a + b[u:u + FT]).astype(BF16)
            if n == NT - 1:
                out_copy(t).start()
        return run

    n_sub = S // SUB
    per_blk = BLK // SUB
    val = [[(("val", t, n), SUB * 5 // 4, (), values(t, n)) for n in range(NT)]
           for t in range(n_sub)]
    inv = [[(("inv", i, c, r), 64, (("bfly", i, c, 3),), inverse(i, c, r))
            for c in range(NT) for r in range(R)] for i in range(NB)]
    bfly = [[(("bfly", i, c, part), 20, (("inv", i - 2, c, R - 1),), inverse_butterfly(i, c, part))
             for c in range(NT) for part in range(4)] for i in range(NB)]
    fin = [[(("fin", t, n), SUB * 5 // 4, (("att", (t + 1) * SUB - AT, TILES[-1]),), finish(t, n))
            for n in range(NT)] for t in range(n_sub)]
    vpu = logit_tasks(-1, S - (P1 or LAG), P1 or LAG) + bfly[0][:-4]
    if not P1:
        vpu += pointwise_tasks(NT - 1)
    soft = [(("soft", u), ST * 5 // 2, (), softmax(u)) for u in range(0, S, ST)]
    vpu += bfly[0][-4:] + soft[:SUB // ST]
    mxu = [task for t in range(LEAD) for task in val[t]]
    mxu[NT:NT] = inv[0][:-R]
    mxu += inv[0][-R:]
    for t in range(n_sub):
        i, sub = divmod(t, per_blk)
        vpu += soft[(t + 1) * SUB // ST:(t + 2) * SUB // ST]
        vpu += [(("att", u, tiles), AT * len(tiles) // 2, (("val", t, NT - 1),), attend(u, tiles))
                for u in range(t * SUB, (t + 1) * SUB, AT) for tiles in TILES]
        if t + LEAD < n_sub:
            mxu += val[t + LEAD]
        if i + 1 < NB:
            vpu += bfly[i + 1][sub * NT:(sub + 1) * NT]
            mxu += inv[i + 1][max(sub * NT - R, 0):(sub + 1) * NT - R * (sub + 1 < per_blk)]
        mxu += fin[t]
    vpu.append((("slack",), SLACK, (), lambda: None))
    paced.clear()
    _interleave(mxu, vpu)
    for t in range(n_sub):
        out_copy(t).wait()


@jax.jit
def pallas_gated_mix__ssm_conv_h3__sliding_local_dilated__prompt_kernel(
    A_q: jax.Array,
    A_k: jax.Array,
    A_v: jax.Array,
    A_shift_k: jax.Array,
    A_ssm_k: jax.Array,
    A_ssm_D: jax.Array,
    B_x: jax.Array,
    B_wqkv: jax.Array,
    B_wo: jax.Array,
    gate_w: jax.Array,
):
    del B_x
    fwd, inv = _dft_tables()
    hbm = pl.BlockSpec(memory_space=pl.ANY)
    vmem = pl.BlockSpec(memory_space=pltpu.VMEM)
    scratch = [
        pltpu.VMEM((NT, S, 128), BF16),
        pltpu.VMEM((2 * NT + 1, PAD + S, 128), BF16),
        pltpu.VMEM((NT, 128, S), BF16),
        pltpu.VMEM((NT, 128, 2 * D), BF16),
        pltpu.VMEM((NT, 128, D), BF16),
        pltpu.VMEM((NT, D, 128), BF16),
        pltpu.VMEM((S, D), BF16),
        pltpu.VMEM((R, 256, 128), BF16),
        pltpu.VMEM((R, 2, 128, 128), BF16),
        pltpu.VMEM((2, D, 128), F32),
        pltpu.VMEM((NT, D // 2, 128), U32),
        pltpu.VMEM((NT, D, 128), U32),
        pltpu.VMEM((NT, D // 2, 128), U32),
        pltpu.VMEM((NT, KS + 2, 8, 128), F32),
        pltpu.VMEM((S // 2, 128), U32),
        pltpu.VMEM((NB, R, 64, 128), U32),
        pltpu.VMEM((6, NB, R, 256, 128), F32),
        pltpu.VMEM((6, NB, R, 256, 128), F32),
        pltpu.VMEM((NT, 2, R, 128, 128), U32),
        pltpu.VMEM((NT, S + 8, 128), F32),
        pltpu.VMEM((NT, HALO + S, 128), F32),
        pltpu.VMEM((W, S, 128), F32),
        pltpu.VMEM((W, S, 128), F32),
        pltpu.VMEM((NT, HALO + S, 128), F32),
        pltpu.VMEM((NT + 1, S + 8, 128), F32),
        pltpu.VMEM((NT, S // 2, 128), U32),
        pltpu.SemaphoreType.DMA((len(HEAD_CHUNKS),)),
        pltpu.SemaphoreType.DMA((2 * NT + 2,)),
        pltpu.SemaphoreType.DMA((NT,)),
        pltpu.SemaphoreType.DMA((S // SUB,)),
    ]
    return pl.pallas_call(
        _kernel,
        out_shape=jax.ShapeDtypeStruct((1, S, D), BF16),
        in_specs=[hbm, hbm, hbm, vmem, hbm, vmem, hbm, hbm, vmem, hbm, hbm,
                  pl.BlockSpec(memory_space=pltpu.SMEM)],
        out_specs=hbm,
        scratch_shapes=scratch,
        compiler_params=pltpu.CompilerParams(vmem_limit_bytes=112 * 1024 * 1024, flags=FLAGS),
    )(A_q, A_k, A_v, A_shift_k.T, A_ssm_k, A_ssm_D, B_wqkv, B_wo, gate_w, fwd, inv,
      np.zeros((3,), np.int32))
```

```python
import numpy as np
import jax
import jax.numpy as jnp
from jax import lax
from jax.experimental import pallas as pl
from jax.experimental.pallas import tpu as pltpu

S = 2048
D = 640
NT = D // 128
KS = 4
H = 32
DH = D // H
W = 8
DIL = 2
R = 4
BLK = 128 * R
NB = S // BLK
HALO = 16
P0 = 416
HEAD_CHUNKS = ((0, 128), (128, 144), (272, 144))
P1 = 192
RS = (S - P0 - P1) // NT
CHUNKS = ((0, 144), (144, 144))
LAG = 144
PAD = 16
QT = 16
HEAD = 4
GAP = 2
EARLY = 3
REST = 250
PACE = ("kv", "q")
IDLE = 100
FM = 256
SUB = 128
AT = 16
FT = 32
LEAD = 3
SLACK = 900
LOG2E = 1.4426950408889634

F32 = jnp.float32
BF16 = jnp.bfloat16
U32 = jnp.uint32


def _dft_tables():
    k = np.concatenate([np.arange(0, 128, 2), np.arange(1, 128, 2)]).astype(np.float64)
    u = np.arange(128, dtype=np.float64)
    fwd = []
    for r in range(R):
        th = 2.0 * np.pi * np.outer(k + 0.5, R * u + r) / (2 * BLK)
        fwd.append(np.stack([np.cos(th).reshape(16, 8, 128), -np.sin(th).reshape(16, 8, 128)],
                            axis=1).reshape(256, 128))
    fwd = np.stack(fwd)
    fwd_in = fwd.reshape(R, 256, 8, 2, 8).transpose(0, 1, 2, 4, 3).reshape(R, 256, 128)
    inv = fwd.reshape(R, 16, 2, 8, 128).transpose(0, 1, 3, 2, 4).reshape(R, 2, 128, 128)
    inv = np.transpose(inv, (0, 1, 3, 2)) / BLK
    return fwd_in.astype(np.float32).astype(BF16), inv.astype(np.float32).astype(BF16)


def _radix4(e, sign):
    (ar, ai), (br, bi), (cr, ci), (dr, di) = e
    s0r, s0i, d0r, d0i = ar + cr, ai + ci, ar - cr, ai - ci
    s1r, s1i, d1r, d1i = br + dr, bi + di, br - dr, bi - di
    plus = (d0r - d1i, d0i + d1r)
    minus = (d0r + d1i, d0i - d1r)
    o1, o3 = (minus, plus) if sign < 0 else (plus, minus)
    return [(s0r + s1r, s0i + s1i), o1, (s0r - s1r, s0i - s1i), o3]


def _interleave(*streams):
    todo = [list(st) for st in streams]
    total = [sum(t[1] for t in st) or 1 for st in streams]
    names = {t[0] for st in streams for t in st}
    spent = [0] * len(streams)
    done = set()
    while any(todo):
        ready = [n for n, st in enumerate(todo)
                 if st and all(d in done or d not in names for d in st[0][2])]
        n = min(ready, key=lambda n: (spent[n] + 0.5 * todo[n][0][1]) / total[n])
        name, cost, _, run = todo[n].pop(0)
        run()
        spent[n] += cost
        done.add(name)


def _load_bf16(ref32, *idx):
    return pltpu.bitcast(ref32[idx], BF16)


def _pack(even, odd):
    return pltpu.pack_elementwise([even, odd], packed_dtype=BF16)


def _unpack(words, index):
    return pltpu.unpack_elementwise(words, index=index, packed_dtype=BF16, unpacked_dtype=F32)


def _kernel(q_hbm, k_hbm, v_hbm, shift_ref, h_hbm, ssmd_ref, wqkv_hbm, wo_hbm, gate_ref,
            fwd_hbm, inv_hbm, zero_ref, out_hbm,
            x_s, kv_s, h_s, wqk_s, wvi_s, wo_s, out_s, fwd_s, inv_s,
            wt_s, wop_s, wc_s, wv_s, par_s, ht_s, dec_s, spec0_s, spec1_s, f_s,
            qa_s, ka_s, p_s, va_s, y_s, o_s,
            sem_x, sem_w, sem_c, sem_o):
    spec_s = (spec0_s, spec1_s)

    def lanes(c):
        return pl.ds(c * 128, 128)

    def x_copies(start, size, sem):
        rows = pl.ds(start, size)
        return [pltpu.make_async_copy(q_hbm.at[0, rows, lanes(kk)], x_s.at[kk, rows], sem)
                for kk in range(NT)]

    def step_copies(c):
        start = P0 + c * RS
        cps = [(h_hbm.at[lanes(c), :], h_s.at[c]),
               (k_hbm.at[0, :, lanes(c)], kv_s.at[c, pl.ds(PAD, S)]),
               (v_hbm.at[0, :, lanes(c)], kv_s.at[NT + c, pl.ds(0, S)]),
               (wqkv_hbm.at[lanes(c), pl.ds(2 * D, D)], wvi_s.at[c]),
               (wo_hbm.at[:, lanes(c)], wo_s.at[c])]
        return (x_copies(start, RS, sem_c.at[c])
                + [pltpu.make_async_copy(src, dst, sem_c.at[c]) for src, dst in cps])

    def w_copy(n):
        kk, part = divmod(n, 2)
        cols = pl.ds(part * D, D)
        return pltpu.make_async_copy(wqkv_hbm.at[lanes(kk), cols], wqk_s.at[kk, :, cols],
                                     sem_w.at[n])

    fwd_copy = pltpu.make_async_copy(fwd_hbm, fwd_s, sem_w.at[2 * NT])
    last_copies = [pltpu.make_async_copy(inv_hbm, inv_s, sem_w.at[2 * NT + 1])]
    if P1:
        last_copies += x_copies(S - P1, P1, sem_w.at[2 * NT + 1])

    head_x = [x_copies(start, size, sem_x.at[n]) for n, (start, size) in enumerate(HEAD_CHUNKS)]
    for cp in (head_x[0] + [w_copy(n) for n in range(2 * NT)] + sum(head_x[1:], [])
               + [fwd_copy] + step_copies(0)):
        cp.start()

    zero, zero_st, zero_pace = zero_ref[0], zero_ref[1], zero_ref[2]

    def spectra(c):
        return spec_s[c % 2].at[zero], spec_s[c % 2].at[zero + 1]

    def z_of(c):
        return spec_s[c % 2].at[zero_st + 2 + c // 2]

    x32 = x_s.bitcast(U32)
    kv32 = kv_s.bitcast(U32)

    paced = []

    def pace(result):
        for name in paced:
            if name == "kv":
                kv32[zero_pace + 2 * NT, pl.ds(S // 2, 8), :] = pltpu.bitcast(result[:8], U32)
            elif name == "q":
                qa_s[zero_pace, pl.ds(S, 8), :] = result[:8]
            else:
                spec_s[name][zero_pace + 5, 0, 0, pl.ds(0, 8), :] = result[:8]
    fwd32 = fwd_s.bitcast(U32)
    inv32 = inv_s.bitcast(U32)

    taps = shift_ref[...].astype(F32)
    ssm_d = ssmd_ref[...].astype(F32).reshape(1, D)
    gate_w = gate_ref[...].astype(F32).reshape(1, D)
    for c in range(NT):
        sl = slice(c * 128, (c + 1) * 128)
        for j in range(KS):
            par_s[c, j] = jnp.broadcast_to(taps[j:j + 1, sl], (8, 128))
        par_s[c, KS] = jnp.broadcast_to(ssm_d[:, sl], (8, 128))
        par_s[c, KS + 1] = jnp.broadcast_to(gate_w[:, sl], (8, 128))

    for c in range(NT):
        ka_s[c, pl.ds(0, HALO), :] = jnp.zeros((HALO, 128), F32)
        kv_s[c, pl.ds(0, PAD), :] = jnp.zeros((PAD, 128), BF16)

    def tile_rows(a, n):
        return jnp.broadcast_to(a[None], (n // 8, 8, 128)).reshape(n, 128)

    def head_rows(ref, start):
        return _pack(ref[pl.ds(start, H // 2, stride=2 * DH), :],
                     ref[pl.ds(start + DH, H // 2, stride=2 * DH), :])

    scale = DH ** -0.5

    for n in range(2 * NT):
        kk, part = divmod(n, 2)
        w_copy(n).wait()
        for j in range(NT):
            wt_s[n % 2, lanes(j), :] = wqk_s[kk, :, lanes(part * NT + j)].astype(F32).T
        for d in range(DH):
            wc_s[kk, pl.ds(part * D // 2 + d * 16, 16), :] = head_rows(wt_s.at[n % 2], d)

    def project(base, size, which, n):
        def run():
            xt = jnp.concatenate([_load_bf16(x32, kk, pl.ds(base // 2, size // 2))
                                  for kk in range(NT)], axis=1)
            wc = jnp.concatenate([_load_bf16(wc_s, kk, pl.ds(which * D // 2 + n * 64, 64))
                                  for kk in range(NT)], axis=1)
            res = lax.dot_general(xt, wc, (((1,), (1,)), ((), ())), preferred_element_type=F32)
            if which == 0:
                qa_s[n, pl.ds(base, size), :] = res
            else:
                ka_s[n, pl.ds(base + HALO, size), :] = res
            pace(res)
        return run

    def logits(base):
        def run():
            qt = [qa_s[n, pl.ds(base, QT), :] for n in range(NT)]
            for w in range(W):
                acc = None
                for n in range(NT):
                    term = qt[n] * ka_s[n, pl.ds(base + (HALO - DIL * w), QT), :]
                    acc = term if acc is None else acc + term
                p_s[w, pl.ds(base, QT), :] = acc
        return run

    def project_tasks(tag, base, size):
        return [(("proj", tag, which, n), size * 5 // 4, (), project(base, size, which, n))
                for which in (1, 0) for n in range(NT)]

    def logit_tasks(tag, base, size):
        return [(("logit", tag, u), 5 * QT // 2, (("proj", tag, 0, NT - 1),), logits(base + u))
                for u in range(0, size, QT)]

    def pointwise(z_s, xs_s, hs_s, g, j):
        def run():
            lo, hi = pl.ds(g * 16, 8), pl.ds(g * 16 + 8, 8)
            xv = [(xs_s[b, j, lo, :], xs_s[b, j, hi, :]) for b in range(NB)]
            hv = [(hs_s[b, j, lo, :], hs_s[b, j, hi, :]) for b in range(NB)]
            hp = [hv[0]]
            for m in range(1, NB):
                if g < 8:
                    hp.append((hv[m][0] - hv[m - 1][1], hv[m][1] + hv[m - 1][0]))
                else:
                    hp.append((hv[m][0] + hv[m - 1][1], hv[m][1] - hv[m - 1][0]))
            for i in range(NB):
                zr = zi = None
                for m in range(i + 1):
                    (hr, hi_), (xr, xi) = hp[m], xv[i - m]
                    pr = hr * xr - hi_ * xi
                    pi = hr * xi + hi_ * xr
                    zr = pr if zr is None else zr + pr
                    zi = pi if zi is None else zi + pi
                z_s[i, j, lo, :] = zr
                z_s[i, j, hi, :] = zi
        return run

    def pointwise_tasks(c):
        return [(("point", g, j), 21, (), pointwise(z_of(c), *spectra(c), g, j))
                for g in range(16) for j in range(R)]

    def tile_step(c):
        base = P0 + c * RS

        def next_inputs():
            for cp in (step_copies(c + 1) if c + 1 < NT else last_copies):
                cp.wait()

        def kv_samples(b, a):
            def run():
                halves = []
                for u in (b * 128 + a * 16, b * 128 + a * 16 + 8):
                    def words(slab, off):
                        return kv32[zero + slab, pl.ds(2 * u + off, 8, stride=2), :]
                    kw = {o: words(c, PAD // 2 + o) for o in (-2, -1, 0, 1)}
                    kt = {t: _unpack(kw[t // 2], t % 2) for t in range(1 - KS, R)}
                    vw = [words(NT + c, o) for o in range(R // 2)]
                    out = []
                    for r in range(R):
                        acc = None
                        for j in range(KS):
                            term = kt[r - j] * par_s[c, j]
                            acc = term if acc is None else acc + term
                        out.append(acc * _unpack(vw[r // 2], r % 2))
                    halves.append(out)
                for r in range(R):
                    kv32[2 * NT, pl.ds((b * R + r) * 64 + a * 8, 8), :] = _pack(
                        halves[0][r], halves[1][r])
            return run

        def h_transpose(t):
            def run():
                ht_s[pl.ds(t * 64, 64), :] = pltpu.bitcast(h_s[c, :, pl.ds(t * 128, 128)].T, U32)
            return run

        def h_samples(b):
            def run():
                for a in range(8):
                    for o in range(R // 2):
                        w0, w1 = (ht_s[pl.ds(2 * (b * 128 + a * 16 + e) + o, 8, stride=2), :]
                                  for e in (0, 8))
                        for e in range(2):
                            dec_s[b, 2 * o + e, pl.ds(a * 8, 8), :] = _pack(
                                _unpack(w0, e), _unpack(w1, e))
            return run

        def forward(slot, dst, b, m):
            def run():
                e = [jnp.dot(_load_bf16(fwd32, r, pl.ds(m * FM // 2, FM // 2)),
                             _load_bf16(dec_s, b, r) if slot else
                             _load_bf16(kv32, 2 * NT, pl.ds((b * R + r) * 64, 64)),
                             preferred_element_type=F32)
                     for r in range(R)]
                for g in range(FM // 16):
                    lo, hi = slice(g * 16, g * 16 + 8), slice(g * 16 + 8, g * 16 + 16)
                    for j, (re, im) in enumerate(_radix4([(er[lo], er[hi]) for er in e], -1)):
                        if slot == 1 and b == 0:
                            re = re + par_s[c, KS]
                        dst[b, j, pl.ds(m * FM + g * 16, 8), :] = re
                        dst[b, j, pl.ds(m * FM + g * 16 + 8, 8), :] = im
                pace(e[-1])
            return run

        def late_weights():
            for n in range(NT):
                wt_s[0, lanes(n), :] = wvi_s[c, :, lanes(n)].astype(F32).T
            wt_s[1] = wo_s[c].astype(F32)
            for d in range(DH):
                wv_s[c, pl.ds(d * 16, 16), :] = head_rows(wt_s.at[0], d)
                wop_s[c, pl.ds(d * 16, 16), :] = head_rows(wt_s.at[1], d)

        proj = sum((project_tasks(n, base + start, size)
                    for n, (start, size) in enumerate(CHUNKS)), [])
        point = pointwise_tasks(c - 1) if c else []
        point.append((("rest",), REST, (), lambda: None))
        xs_s, hs_s = spectra(c)
        logit = logit_tasks(-1, base - LAG, LAG)
        for n, (start, size) in enumerate(CHUNKS):
            logit += logit_tasks(n, base + start, min(size, RS - LAG - start))
        mxu, prep = proj[:HEAD], []
        for b in range(NB):
            prep += [(("ht", t), 10, (), h_transpose(t)) for t in range(4 * b, 4 * b + 4)]
            prep += [(("dec", 1, b), 24, (), h_samples(b))]
            prep += [(("dec", 0, b, a), 24, (), kv_samples(b, a)) for a in range(8)]
            for slot, dst, need in ((1, hs_s, ("dec", 1, b)), (0, xs_s, ("dec", 0, b, 7))):
                mxu += [(("fwd", slot, b, m), FM, (need,), forward(slot, dst, b, m))
                        for m in range(256 // FM)]
                lo = HEAD + (2 * b + 1 - slot) * GAP
                mxu += proj[lo:lo + GAP]
        mxu += proj[HEAD + 2 * NB * GAP:]
        mxu.insert(len(mxu) - EARLY, (("wait",), 0, (("point", 15, R - 1),), next_inputs))
        prep += [(("late",), 150, (), late_weights), (("idle",), IDLE, (), lambda: None)]
        paced[:] = [name for name in ("kv", "q", (c + 1) % 2) if name in PACE or name in (0, 1)]
        _interleave(mxu, prep, point, logit)

    done = 0
    for n, (start, size) in enumerate(HEAD_CHUNKS):
        for cp in head_x[n]:
            cp.wait()
        for c in range(1, NT):
            if (c - 1) * len(HEAD_CHUNKS) // (NT - 1) == n:
                for cp in step_copies(c):
                    cp.start()
        ready = min(start, P0 - LAG)
        _interleave(project_tasks(n, start, size), logit_tasks(-1, done, ready - done))
        done = ready
    _interleave(logit_tasks(-1, done, P0 - LAG - done))
    fwd_copy.wait()
    for cp in last_copies:
        cp.start()
    for cp in step_copies(0):
        cp.wait()
    for c in range(NT):
        tile_step(c)
    if P1:
        paced[:] = [(NT - 1) % 2, "q"]
        _interleave(project_tasks(0, S - P1, P1), pointwise_tasks(NT - 1),
                    logit_tasks(-1, S - P1 - LAG, LAG))

    row = lax.broadcasted_iota(jnp.int32, (HALO, 128), 0)
    for w in range(1, W):
        p_s[w, pl.ds(0, HALO), :] = jnp.where(row < DIL * w, -0.25e9 / scale,
                                              p_s[w, pl.ds(0, HALO), :])

    def out_copy(i):
        rows = pl.ds(i * SUB, SUB)
        return pltpu.make_async_copy(out_s.at[rows, :], out_hbm.at[0, rows, :], sem_o.at[i])

    def inverse(i, c, r):
        def run():
            y = jnp.dot(
                jnp.concatenate([_load_bf16(inv32, r, 0), _load_bf16(inv32, r, 1)], axis=1),
                _load_bf16(f_s, c, i % 2, r), preferred_element_type=F32)
            y_s[c, pl.ds(i * BLK + r, 128, stride=R), :] = y
        return run

    def inverse_butterfly(i, c, part):
        def run():
            z_s = z_of(c)
            for g in range(4 * part, 4 * part + 4):
                z = [(z_s[i, j, pl.ds(g * 16, 8), :], z_s[i, j, pl.ds(g * 16 + 8, 8), :])
                     for j in range(R)]
                for r, (re, im) in enumerate(_radix4(z, +1)):
                    f_s[c, i % 2, r, pl.ds(g * 8, 8), :] = _pack(re, im)
        return run

    def values(t, n):
        def run():
            if n:
                return
            xt = jnp.concatenate([_load_bf16(x32, kk, pl.ds(t * SUB // 2, SUB // 2))
                                  for kk in range(NT)], axis=1)
            wv = jnp.concatenate([_load_bf16(wv_s, kk) for kk in range(NT)], axis=1)
            v = lax.dot_general(xt, wv, (((1,), (1,)), ((), ())), preferred_element_type=F32)
            for c in range(NT):
                tile = v[:, c * 128:(c + 1) * 128]
                va_s[c, pl.ds(HALO + t * SUB, SUB), :] = tile
                if t == 0:
                    va_s[c, pl.ds(0, HALO), :] = jnp.broadcast_to(tile[0:1], (HALO, 128))
        return run

    def attend(u):
        def run():
            half = []
            for par in range(2):
                rows = pl.ds(u + par, AT // 2, stride=2)
                logit = []
                for w in range(W):
                    a = p_s[w, rows, :]
                    a = a + pltpu.roll(a, 64, 1)
                    logit.append(a + pltpu.roll(a, 32, 1))
                m = logit[0]
                for w in range(1, W):
                    m = jnp.maximum(m, logit[w])
                e = [jnp.exp2((l - m) * (scale * LOG2E)) for l in logit]
                den = e[0]
                for w in range(1, W):
                    den = den + e[w]
                inv = pl.reciprocal(den, approx=True)
                inv = inv * (2.0 - den * inv)
                gs = None
                for c in range(NT):
                    term = _unpack(x32[c, pl.ds(u // 2, AT // 2), :], par) * tile_rows(
                        par_s[c, KS + 1], AT // 2)
                    gs = term if gs is None else gs + term
                th = 0.5 * jnp.tanh(0.5 * jnp.sum(gs, axis=1, keepdims=True))
                y_s[NT, rows, :] = jnp.broadcast_to(0.5 + th, (AT // 2, 128))
                inv = inv * (0.5 - th)
                acc = []
                for c in range(NT):
                    a = None
                    for w in range(W):
                        term = e[w] * va_s[c, pl.ds(u + par + HALO - DIL * w, AT // 2, stride=2), :]
                        a = term if a is None else a + term
                    acc.append(a * inv)
                half.append(acc)
            for c in range(NT):
                o_s[c, pl.ds(u // 2, AT // 2), :] = _pack(half[0][c], half[1][c])
        return run

    def finish(t, n):
        def run():
            if n:
                return
            half = pl.ds(t * SUB // 2, SUB // 2)
            o = jnp.concatenate([_load_bf16(o_s, c, half) for c in range(NT)], axis=1)
            wo = jnp.concatenate([_load_bf16(wop_s, c) for c in range(NT)], axis=1)
            b = jnp.dot(o, wo, preferred_element_type=F32)
            for u in range(0, SUB, FT):
                rws = pl.ds(t * SUB + u, FT)
                for c in range(NT):
                    a = x_s[c, rws, :].astype(F32) * y_s[c, rws, :]
                    out_s[rws, lanes(c)] = (
                        y_s[NT, rws, :] * a + b[u:u + FT, c * 128:(c + 1) * 128]).astype(BF16)
            out_copy(t).start()
        return run

    n_sub = S // SUB
    per_blk = BLK // SUB
    val = [[(("val", t, n), SUB * 5 // 4, (), values(t, n)) for n in range(NT)]
           for t in range(n_sub)]
    inv = [[(("inv", i, c, r), 64, (("bfly", i, c, 3),), inverse(i, c, r))
            for c in range(NT) for r in range(R)] for i in range(NB)]
    bfly = [[(("bfly", i, c, part), 20, (("inv", i - 2, c, R - 1),), inverse_butterfly(i, c, part))
             for c in range(NT) for part in range(4)] for i in range(NB)]
    fin = [[(("fin", t, n), SUB * 5 // 4, (("att", (t + 1) * SUB - AT),), finish(t, n))
            for n in range(NT)] for t in range(n_sub)]
    vpu = logit_tasks(-1, S - (P1 or LAG), P1 or LAG) + bfly[0][:-4]
    if not P1:
        vpu += pointwise_tasks(NT - 1)
    vpu += bfly[0][-4:]
    mxu = [task for t in range(LEAD) for task in val[t]]
    mxu[NT:NT] = inv[0][:-R]
    mxu += inv[0][-R:]
    for t in range(n_sub):
        i, sub = divmod(t, per_blk)
        vpu += [(("att", u), AT * 5, (("val", t, NT - 1),), attend(u))
                for u in range(t * SUB, (t + 1) * SUB, AT)]
        if t + LEAD < n_sub:
            mxu += val[t + LEAD]
        if i + 1 < NB:
            vpu += bfly[i + 1][sub * NT:(sub + 1) * NT]
            mxu += inv[i + 1][max(sub * NT - R, 0):(sub + 1) * NT - R * (sub + 1 < per_blk)]
        mxu += fin[t]
    vpu.append((("slack",), SLACK, (), lambda: None))
    paced.clear()
    _interleave(mxu, vpu)
    for t in range(n_sub):
        out_copy(t).wait()


@jax.jit
def pallas_gated_mix__ssm_conv_h3__sliding_local_dilated__prompt_kernel(
    A_q: jax.Array,
    A_k: jax.Array,
    A_v: jax.Array,
    A_shift_k: jax.Array,
    A_ssm_k: jax.Array,
    A_ssm_D: jax.Array,
    B_x: jax.Array,
    B_wqkv: jax.Array,
    B_wo: jax.Array,
    gate_w: jax.Array,
):
    del B_x
    fwd, inv = _dft_tables()
    hbm = pl.BlockSpec(memory_space=pl.ANY)
    vmem = pl.BlockSpec(memory_space=pltpu.VMEM)
    scratch = [
        pltpu.VMEM((NT, S, 128), BF16),
        pltpu.VMEM((2 * NT + 1, PAD + S, 128), BF16),
        pltpu.VMEM((NT, 128, S), BF16),
        pltpu.VMEM((NT, 128, 2 * D), BF16),
        pltpu.VMEM((NT, 128, D), BF16),
        pltpu.VMEM((NT, D, 128), BF16),
        pltpu.VMEM((S, D), BF16),
        pltpu.VMEM((R, 256, 128), BF16),
        pltpu.VMEM((R, 2, 128, 128), BF16),
        pltpu.VMEM((2, D, 128), F32),
        pltpu.VMEM((NT, D // 2, 128), U32),
        pltpu.VMEM((NT, D, 128), U32),
        pltpu.VMEM((NT, D // 2, 128), U32),
        pltpu.VMEM((NT, KS + 2, 8, 128), F32),
        pltpu.VMEM((S // 2, 128), U32),
        pltpu.VMEM((NB, R, 64, 128), U32),
        pltpu.VMEM((6, NB, R, 256, 128), F32),
        pltpu.VMEM((6, NB, R, 256, 128), F32),
        pltpu.VMEM((NT, 2, R, 128, 128), U32),
        pltpu.VMEM((NT, S + 8, 128), F32),
        pltpu.VMEM((NT, HALO + S, 128), F32),
        pltpu.VMEM((W, S, 128), F32),
        pltpu.VMEM((NT, HALO + S, 128), F32),
        pltpu.VMEM((NT + 1, S + 8, 128), F32),
        pltpu.VMEM((NT, S // 2, 128), U32),
        pltpu.SemaphoreType.DMA((len(HEAD_CHUNKS),)),
        pltpu.SemaphoreType.DMA((2 * NT + 2,)),
        pltpu.SemaphoreType.DMA((NT,)),
        pltpu.SemaphoreType.DMA((S // SUB,)),
    ]
    return pl.pallas_call(
        _kernel,
        out_shape=jax.ShapeDtypeStruct((1, S, D), BF16),
        in_specs=[hbm, hbm, hbm, vmem, hbm, vmem, hbm, hbm, vmem, hbm, hbm,
                  pl.BlockSpec(memory_space=pltpu.SMEM)],
        out_specs=hbm,
        scratch_shapes=scratch,
        compiler_params=pltpu.CompilerParams(vmem_limit_bytes=112 * 1024 * 1024),
    )(A_q, A_k, A_v, A_shift_k.T, A_ssm_k, A_ssm_D, B_wqkv, B_wo, gate_w, fwd, inv,
      np.zeros((3,), np.int32))
```
